```python
import jax
import jax.numpy as jnp

def _softmax(x, axis=-1):
    return jax.nn.softmax(x, axis=axis)
def _gelu(x):
    return jax.nn.gelu(x, approximate=True)
def _silu(x):
    return jax.nn.silu(x)
def _sigmoid(x):
    return jax.nn.sigmoid(x)
def _layernorm(x, axis=-1, eps=1e-5):
    m = jnp.mean(x, axis=axis, keepdims=True)
    v = jnp.var(x, axis=axis, keepdims=True)
    return (x - m) / jnp.sqrt(v + eps)
def _scatter_add(tgt, idx, src, axis=0):
    return tgt.at[idx].add(src)
def _segment_sum(src, seg, n):
    return jax.ops.segment_sum(src, seg, n)
class _Rng:
    def __init__(self, key):
        self._k = key
    def _next(self):
        self._k, sub = jax.random.split(self._k)
        return sub
    def normal(self, shape):
        return jax.random.normal(self._next(), shape, dtype=jnp.bfloat16)
    def randint(self, lo, hi, shape):
        return jax.random.randint(self._next(), shape, lo, hi, dtype=jnp.int32)
    def uniform(self, shape, lo=0.0, hi=1.0):
        return jax.random.uniform(self._next(), shape, jnp.bfloat16, lo, hi)
    def permutation(self, n):
        return jax.random.permutation(self._next(), n)


kernel_name = 'standalone__gqa_block_cached__near_ridge'

def setup_inputs():
    _rng = _Rng(jax.random.key(int.from_bytes(__import__("os").urandom(4), "little")))
    _w = (lambda a: (lambda t: t.astype(jnp.bfloat16) if jnp.issubdtype(t.dtype, jnp.floating) else t)(jnp.asarray(a)))
    B, Sq, D = 16, 240, 640
    Hq, Hkv, Sk, Dh = 32, 32, 1024, 128
    assert Hq % Hkv == 0, (Hq, Hkv)
    return {
        "x": _w((lambda *s: _rng.normal(s) * 0.05)(B, Sq, D)),
        "k_cache": _w((lambda *s: _rng.normal(s) * 0.05)(B, Hkv, Sk, Dh)),
        "v_cache": _w((lambda *s: _rng.normal(s) * 0.05)(B, Hkv, Sk, Dh)),
        "wq": _w((lambda *s: _rng.normal(s) * 0.05)(D, Hq * Dh) * (D ** -0.5)),
        "wo": _w((lambda *s: _rng.normal(s) * 0.05)(Hq * Dh, D) * ((Hq * Dh) ** -0.5)),
    }

def reference(x, k_cache, v_cache, wq, wo):
    B, Sq, D = x.shape
    Hq, Dh = 32, 128
    Hkv = k_cache.shape[1]
    rep = Hq // Hkv
    q = (lambda x, *d: x.transpose(*d))((x @ wq).reshape(B, Sq, Hq, Dh), 0, 2, 1, 3)
    k = jnp.repeat(k_cache, rep, axis=1)
    v = jnp.repeat(v_cache, rep, axis=1)
    scores = jnp.einsum("bhqd,bhkd->bhqk", q, k) * (Dh ** -0.5)
    p = _softmax(scores, axis=-1)
    o = jnp.einsum("bhqk,bhkd->bhqd", p, v)
    return (lambda x, *d: x.transpose(*d))(o, 0, 2, 1, 3).reshape(B, Sq, Hq * Dh) @ wo
```

```python
import functools

import jax
import jax.numpy as jnp
import jax.experimental.pallas as pl
import jax.experimental.pallas.tpu as pltpu

_G = 4


def _kernel(x_ref, k_ref, v_ref, wq_ref, wo_ref, o_ref, acc_ref, *, G, Dh):
    g = pl.program_id(1)
    x = x_ref[0]
    col = pl.multiple_of(g * (G * Dh), G * Dh)
    q = jnp.dot(x, wq_ref[:, pl.ds(col, G * Dh)], preferred_element_type=jnp.float32)
    q = (q * (Dh ** -0.5)).astype(jnp.bfloat16)
    outs = []
    for h in range(G):
        qh = q[:, h * Dh:(h + 1) * Dh]
        s = jax.lax.dot_general(qh, k_ref[0, h], (((1,), (1,)), ((), ())),
                                preferred_element_type=jnp.float32)
        m = jnp.max(s, axis=-1, keepdims=True)
        p = jnp.exp(s - m)
        l = jnp.sum(p, axis=-1, keepdims=True)
        o = jnp.dot(p.astype(jnp.bfloat16), v_ref[0, h], preferred_element_type=jnp.float32)
        outs.append((o / l).astype(jnp.bfloat16))
    o = jnp.concatenate(outs, axis=-1)
    y = jnp.dot(o, wo_ref[pl.ds(col, G * Dh), :], preferred_element_type=jnp.float32)

    @pl.when(g == 0)
    def _():
        acc_ref[...] = y

    @pl.when(g > 0)
    def _():
        acc_ref[...] += y

    @pl.when(g == pl.num_programs(1) - 1)
    def _():
        o_ref[0] = acc_ref[...].astype(o_ref.dtype)


@jax.jit
def pallas_standalone__gqa_block_cached__near_ridge_kernel(x, k_cache, v_cache, wq, wo):
    B, Sq, D = x.shape
    _, Hkv, Sk, Dh = k_cache.shape
    G = _G
    return pl.pallas_call(
        functools.partial(_kernel, G=G, Dh=Dh),
        grid=(B, Hkv // G),
        in_specs=[
            pl.BlockSpec((1, Sq, D), lambda b, g: (b, 0, 0)),
            pl.BlockSpec((1, G, Sk, Dh), lambda b, g: (b, g, 0, 0)),
            pl.BlockSpec((1, G, Sk, Dh), lambda b, g: (b, g, 0, 0)),
            pl.BlockSpec(wq.shape, lambda b, g: (0, 0)),
            pl.BlockSpec(wo.shape, lambda b, g: (0, 0)),
        ],
        out_specs=pl.BlockSpec((1, Sq, D), lambda b, g: (b, 0, 0)),
        out_shape=jax.ShapeDtypeStruct((B, Sq, D), x.dtype),
        scratch_shapes=[pltpu.VMEM((Sq, D), jnp.float32)],
        compiler_params=pltpu.CompilerParams(
            dimension_semantics=("arbitrary", "arbitrary"),
            vmem_limit_bytes=100 * 1024 * 1024,
        ),
    )(x, k_cache, v_cache, wq, wo)
```

```python
import functools
import math

import jax
import jax.numpy as jnp
import jax.experimental.pallas as pl
import jax.experimental.pallas.tpu as pltpu

_G = 8
_RC = 16
_NS = 2
_NB = 2
_CH = 1
_RT = 3
_KVAT = 1
_L = 128


def _plan(G, NC, ND):
    o_r = [("o", j, n) for j in range(G // 4) for n in range(ND)]
    q_r = [("q", j, n) for j in range(G // 4) for n in range(ND)]
    proj = o_r + q_r
    gaps = [int(c) for c in "323232320"]
    assert len(gaps) == G + 1 and sum(gaps) == len(proj)
    rounds, done = [], 0
    for h in range(G):
        rounds += [("qk", h, 0), ("qk", h, 1)]
        if h > 0:
            rounds += [("pv", h - 1, 0), ("pv", h - 1, 1)]
        rounds += proj[done:done + gaps[h]]
        done += gaps[h]
    rounds += [("pv", G - 1, 0), ("pv", G - 1, 1)] + proj[done:]
    pos = {r: i for i, r in enumerate(rounds)}
    for j in range(G // 4):
        assert pos[("q", j, ND - 1)] > pos[("qk", 4 * j + 3, 1)]
    first = [pos[("qk", h, 1)] for h in range(G)]
    last = [pos[("pv", h, 0)] - 1 for h in range(G)]
    after = [[] for _ in rounds]
    left = [NC] * G
    for i in range(len(rounds)):
        rate, tot = 0.0, 0
        for h in range(G):
            if left[h] and first[h] <= i:
                tot += left[h]
                rate = max(rate, tot / (last[h] - i + 1))
        n = math.ceil(rate - 1e-9)
        for h in range(G):
            while n and left[h] and first[h] <= i:
                after[i].append((h, NC - left[h]))
                left[h] -= 1
                n -= 1
    assert not any(left)
    return rounds, after


def _dot(a, b, transpose_b=False):
    dims = (((1,), (1 if transpose_b else 0,)), ((), ()))
    return jax.lax.dot_general(a, b, dims, preferred_element_type=jnp.float32)


def _cat(xs, axis):
    return jnp.concatenate(list(xs), axis=axis)


def _kernel(x_hbm, k_hbm, v_hbm, wq_hbm, wo_hbm, out_hbm,
            x_ref, k_ref, v_ref, wq_ref, wo_ref, o_ref, q_buf, o_buf, acc_ref, qacc_ref, oacc_ref, s_buf, p_buf, r_buf,
            x_sem, k_sem, v_sem, wq_sem, wo_sem, o_sem, *, G):
    B, Sq, D = x_ref.shape
    ND = D // _L
    NB, _, Sk, Dh = k_ref.shape
    NG = k_hbm.shape[1] // G
    T = B * NG
    W = G * Dh
    NS, NK = s_buf.shape[:2]
    HK = Sk // 2
    scale = Dh ** -0.5 * math.log2(math.e)
    f32 = jnp.float32

    def x_copies(b):
        return [pltpu.make_async_copy(x_hbm.at[b], x_ref.at[b], x_sem.at[b])]

    def kv_copies(step):
        slot, step = step % NB, jnp.minimum(step, T - 1)
        src = step // NG, pl.ds((step % NG) * G, G)
        return (pltpu.make_async_copy(k_hbm.at[src], k_ref.at[slot], k_sem.at[slot]),
                pltpu.make_async_copy(v_hbm.at[src], v_ref.at[slot], v_sem.at[slot]))

    def wq_copies(g):
        cols = pl.ds(pl.multiple_of(g * W, W), W)
        return [pltpu.make_async_copy(wq_hbm.at[:, cols], wq_ref.at[:, cols], wq_sem.at[g])]

    def wo_copies(g):
        rows = pl.ds(pl.multiple_of(g * W, W), W)
        return [pltpu.make_async_copy(wo_hbm.at[rows], wo_ref.at[rows], wo_sem.at[g])]

    def out_copies(b):
        return [pltpu.make_async_copy(o_ref.at[b], out_hbm.at[b], o_sem.at[b])]

    def start(cps):
        for cp in cps:
            cp.start()

    def wait(cps):
        for cp in cps:
            cp.wait()

    def q_round(step, j, n):
        col = pl.multiple_of(((step % NG) * G + 4 * j) * Dh, 4 * Dh)
        ks = slice(n * _L, (n + 1) * _L)
        q = _dot(x_ref[step // NG, :, ks], wq_ref[ks, pl.ds(col, 4 * Dh)])
        for i in range(4):
            qi = q[:, i * Dh:(i + 1) * Dh]
            if n > 0:
                qi = qi + qacc_ref[i]
            if n < ND - 1:
                qacc_ref[i] = qi
            else:
                q_buf[4 * j + i] = (qi * scale).astype(q_buf.dtype)

    def o_round(step, j, n, o_prev):
        grp = step % NG
        row = pl.multiple_of((grp * G + 4 * j) * Dh, 4 * Dh)
        y = _dot(_cat(o_prev[4 * j:4 * j + 4], 1), wo_ref[pl.ds(row, 4 * Dh), n * _L:(n + 1) * _L])
        acc = acc_ref[n] + y
        if j == 0:
            acc = jnp.where(grp == 0, y, acc)
        acc_ref[n] = acc
        if j == G // 4 - 1:
            o_ref[step // NG, :, n * _L:(n + 1) * _L] = acc.astype(o_ref.dtype)

    mpart, lsum, rcp = {}, {}, {}

    def qk_round(slot, h, c):
        s = _dot(q_buf[h], k_ref[slot, h, c * HK:(c + 1) * HK, :], transpose_b=True)
        s = [s[:, i * _L:(i + 1) * _L] for i in range(NK // 2)]
        for i, si in enumerate(s):
            s_buf[h % NS, c * (NK // 2) + i] = si
        m = functools.reduce(jnp.maximum, s)
        if c == 0:
            mpart[h] = m
        else:
            mpart[h] = jnp.max(jnp.maximum(m, mpart[h]), axis=-1, keepdims=True)

    def softmax(never, h, c):
        rs = slice(c * _RC, (c + 1) * _RC)
        m = mpart[h][rs]
        if (h, c - _RT) in rcp:
            m = jnp.where(never, rcp[h, c - _RT], m)
        if (h, c - _CH) in lsum:
            m = jnp.where(never, lsum[h, c - _CH], m)
        p = [jnp.exp2(s_buf[h % NS, i, rs, :] - m) for i in range(NK)]
        lp = functools.reduce(jnp.add, p)
        lsum[h, c] = lp
        p[-1] = jnp.where(never, lp, p[-1])
        for i, pi in enumerate(p):
            p_buf[h % NS, i, rs, :] = pi.astype(p_buf.dtype)
        l = jnp.sum(lp, axis=-1, keepdims=True)
        r = pl.reciprocal(l, approx=True)
        r = r * (2.0 - l * r)
        rcp[h, c] = r
        r_buf[h % NS, rs, :] = jnp.broadcast_to(r, (_RC, Dh))

    def pv_round(slot, h, c):
        p = _cat((p_buf[h % NS, c * (NK // 2) + i] for i in range(NK // 2)), 1)
        o = _dot(p, v_ref[slot, h, c * HK:(c + 1) * HK, :])
        if c == 0:
            oacc_ref[...] = o
        else:
            o_buf[h] = ((o + oacc_ref[...]) * r_buf[h % NS]).astype(o_buf.dtype)

    start(x_copies(0))
    start(wq_copies(0))
    start(kv_copies(0))
    start(wo_copies(0))
    start(wq_copies(1))
    start(x_copies(1))
    for s in range(1, NB - 1):
        start(kv_copies(s))

    wait(x_copies(0))
    wait(wq_copies(0))
    for j in range(G // 4):
        for n in range(ND):
            q_round(0, j, n)
    o_buf[...] = jnp.zeros_like(o_buf)
    acc_ref[...] = jnp.zeros_like(acc_ref)
    wait(wo_copies(0))
    rounds, after = _plan(G, Sq // _RC, ND)

    def step(t, _):
        @pl.when(t <= NG)
        def _():
            @pl.when(t + 1 < NG)
            def _():
                start(wo_copies(t + 1))

            @pl.when(t + 2 < NG)
            def _():
                start(wq_copies(t + 2))

            @pl.when(t + 1 < NG)
            def _():
                wait(wq_copies(t + 1))

            @pl.when(t >= 2)
            def _():
                wait(wo_copies(t - 1))

        @pl.when(t % NG == NG - 1)
        def _():
            b = t // NG

            @pl.when(b + 2 < B)
            def _():
                start(x_copies(b + 2))

            @pl.when(b + 1 < B)
            def _():
                wait(x_copies(b + 1))

            @pl.when(b > 0)
            def _():
                start(out_copies(b - 1))

        wait(kv_copies(t))
        prev = jnp.maximum(t - 1, 0)
        nxt = jnp.minimum(t + 1, T - 1)
        slot = t % NB
        o_prev = [o_buf[h] for h in range(G)]
        for i, ((kind, a, b), chunks) in enumerate(zip(rounds, after)):
            if i == _KVAT:
                start(kv_copies(t + NB - 1))
            if kind == "qk":
                qk_round(slot, a, b)
            elif kind == "pv":
                pv_round(slot, a, b)
            elif kind == "o":
                o_round(prev, a, b, o_prev)
            else:
                q_round(nxt, a, b)
            for h, c in chunks:
                softmax(t < 0, h, c)

    jax.lax.fori_loop(0, T, step, None)
    o_prev = [o_buf[h] for h in range(G)]
    for j in range(G // 4):
        for n in range(ND):
            o_round(T - 1, j, n, o_prev)
    start(out_copies(B - 1))
    for s in range(NB - 1):
        wait(kv_copies(T + s))
    for b in range(B):
        wait(out_copies(b))


@jax.jit
def pallas_standalone__gqa_block_cached__near_ridge_kernel(x, k_cache, v_cache, wq, wo):
    B, Sq, D = x.shape
    _, Hkv, Sk, Dh = k_cache.shape
    G, NS, NB = _G, _NS, _NB
    NG, ND, NK = Hkv // G, D // _L, Sk // _L
    bf16, f32 = jnp.bfloat16, jnp.float32
    DMA = pltpu.SemaphoreType.DMA
    return pl.pallas_call(
        functools.partial(_kernel, G=G),
        in_specs=[pl.BlockSpec(memory_space=pl.ANY)] * 5,
        out_specs=pl.BlockSpec(memory_space=pl.ANY),
        out_shape=jax.ShapeDtypeStruct((B, Sq, D), x.dtype),
        scratch_shapes=[
            pltpu.VMEM(x.shape, x.dtype),
            pltpu.VMEM((NB, G, Sk, Dh), k_cache.dtype),
            pltpu.VMEM((NB, G, Sk, Dh), v_cache.dtype),
            pltpu.VMEM(wq.shape, wq.dtype),
            pltpu.VMEM(wo.shape, wo.dtype),
            pltpu.VMEM(x.shape, x.dtype),
            pltpu.VMEM((G, Sq, Dh), bf16),
            pltpu.VMEM((G, Sq, Dh), bf16),
            pltpu.VMEM((ND, Sq, _L), f32),
            pltpu.VMEM((4, Sq, Dh), f32),
            pltpu.VMEM((Sq, Dh), f32),
            pltpu.VMEM((NS, NK, Sq, _L), f32),
            pltpu.VMEM((NS, NK, Sq, _L), bf16),
            pltpu.VMEM((NS, Sq, Dh), f32),
            DMA((B,)), DMA((NB,)), DMA((NB,)), DMA((NG,)), DMA((NG,)), DMA((B,)),
        ],
        compiler_params=pltpu.CompilerParams(
            vmem_limit_bytes=100 * 1024 * 1024,
            disable_bounds_checks=True,
        ),
    )(x, k_cache, v_cache, wq, wo)
```

```python
import functools
import math

import jax
import jax.numpy as jnp
import jax.experimental.pallas as pl
import jax.experimental.pallas.tpu as pltpu

_G = 16
_RB = 16
_R0 = 6
_KC = 4
_NB = 2 * _G // _KC
_RC = 16
_NS = 2
_CH = 1
_RT = 2
_EARLY = 2
_L = 128


def _plan(G, NC, ND):
    gaps = [int(c) for c in "3322"]
    assert len(gaps) == 4 and sum(gaps) == 2 * ND
    rounds = []
    for j in range(G // 4):
        proj = [("q", j, n) for n in range(ND)] + [("o", j, n) for n in range(ND)]
        for i in range(4):
            h = 4 * j + i
            rounds += [("qk", h, 0), ("qk", h, 1)]
            if h > 0:
                rounds += [("pv", h - 1, 0), ("pv", h - 1, 1)]
            rounds += proj[sum(gaps[:i]):sum(gaps[:i + 1])]
    rounds += [("pv", G - 1, 0), ("pv", G - 1, 1)]
    pos = {r: i for i, r in enumerate(rounds)}
    first = [pos[("qk", h, 1)] for h in range(G)]
    last = [pos[("pv", h, 0)] - 1 for h in range(G)]
    after = [[] for _ in rounds]
    left = [NC] * G
    for i in range(len(rounds)):
        rate, tot = 0.0, 0
        for h in range(G):
            if left[h] and first[h] <= i:
                tot += left[h]
                rate = max(rate, tot / (last[h] - i + 1))
        n = math.ceil(rate - 1e-9)
        for h in range(G):
            while n and left[h] and first[h] <= i:
                after[i].append((h, NC - left[h]))
                left[h] -= 1
                n -= 1
    assert not any(left)
    return rounds, after


def _dot(a, b, transpose_b=False):
    dims = (((1,), (1 if transpose_b else 0,)), ((), ()))
    return jax.lax.dot_general(a, b, dims, preferred_element_type=jnp.float32)


def _cat(xs, axis):
    return jnp.concatenate(list(xs), axis=axis)


def _kernel(x_hbm, k_hbm, v_hbm, wq_hbm, wo_hbm, out_hbm,
            x_ref, k_ref, v_ref, wq_ref, wo_ref, o_ref, q_buf, o_buf, acc_ref, qacc_ref, oacc_ref, s_buf, p_buf, r_buf,
            x_sem, k_sem, v_sem, wq_sem, wo_sem, o_sem, *, G):
    B, Sq, D = x_ref.shape
    ND = D // _L
    NB, KC, Sk, Dh = k_ref.shape
    H = k_hbm.shape[1]
    NG, NCH = H // 4, H // KC
    W = 4 * Dh
    NS, NK = s_buf.shape[:2]
    HK = Sk // 2
    scale = Dh ** -0.5 * math.log2(math.e)
    f32 = jnp.float32

    def x_copy(b):
        return pltpu.make_async_copy(x_hbm.at[b], x_ref.at[b], x_sem.at[b])

    def kv_copy(hbm, ref, sem, c):
        slot = c % NB
        return pltpu.make_async_copy(hbm.at[c // NCH, pl.ds((c % NCH) * KC, KC)], ref.at[slot], sem.at[slot])

    k_copy = functools.partial(kv_copy, k_hbm, k_ref, k_sem)
    v_copy = functools.partial(kv_copy, v_hbm, v_ref, v_sem)

    def wq_copy(g):
        cols = pl.ds(pl.multiple_of(g * W, W), W)
        return pltpu.make_async_copy(wq_hbm.at[:, cols], wq_ref.at[:, cols], wq_sem.at[g])

    def wo_copy(g):
        rows = pl.ds(pl.multiple_of(g * W, W), W)
        return pltpu.make_async_copy(wo_hbm.at[rows], wo_ref.at[rows], wo_sem.at[g])

    def out_copy(b):
        return pltpu.make_async_copy(o_ref.at[b], out_hbm.at[b], o_sem.at[b])

    def q_round(g, par, n):
        col = pl.multiple_of((g % NG) * W, W)
        ks = slice(n * _L, (n + 1) * _L)
        q = _dot(x_ref[g // NG, :, ks], wq_ref[ks, pl.ds(col, W)])
        for i in range(4):
            qi = q[:, i * Dh:(i + 1) * Dh]
            if n > 0:
                qi = qi + qacc_ref[i]
            if n < ND - 1:
                qacc_ref[i] = qi
            else:
                q_buf[4 * par + i] = (qi * scale).astype(q_buf.dtype)

    def o_round(g, par, n, maybe_first, maybe_last):
        row = pl.multiple_of((g % NG) * W, W)
        cs = slice(n * _L, (n + 1) * _L)
        y = _dot(_cat((o_buf[4 * par + i] for i in range(4)), 1), wo_ref[pl.ds(row, W), cs])
        acc = acc_ref[n] + y
        if maybe_first:
            acc = jnp.where(g % NG == 0, y, acc)
        acc_ref[n] = acc
        if maybe_last:
            o_ref[g // NG, :, cs] = acc.astype(o_ref.dtype)

    mpart, lsum, rcp = {}, {}, {}

    def qk_round(slot, h, c):
        s = _dot(q_buf[h], k_ref[slot, h % KC, c * HK:(c + 1) * HK, :], transpose_b=True)
        s = [s[:, i * _L:(i + 1) * _L] for i in range(NK // 2)]
        for i, si in enumerate(s):
            s_buf[h % NS, c * (NK // 2) + i] = si
        m = functools.reduce(jnp.maximum, s)
        if c == 0:
            mpart[h] = m
        else:
            mpart[h] = jnp.max(jnp.maximum(m, mpart[h]), axis=-1, keepdims=True)

    def softmax(never, h, c):
        rs = slice(c * _RC, (c + 1) * _RC)
        m = mpart[h][rs]
        if (h, c - _RT) in rcp:
            m = jnp.where(never, rcp[h, c - _RT], m)
        if (h, c - _CH) in lsum:
            m = jnp.where(never, lsum[h, c - _CH], m)
        p = [jnp.exp2(s_buf[h % NS, i, rs, :] - m) for i in range(NK)]
        lp = functools.reduce(jnp.add, p)
        lsum[h, c] = lp
        p[-1] = jnp.where(never, lp, p[-1])
        for i, pi in enumerate(p):
            p_buf[h % NS, i, rs, :] = pi.astype(p_buf.dtype)
        l = jnp.sum(lp, axis=-1, keepdims=True)
        r = pl.reciprocal(l, approx=True)
        r = r * (2.0 - l * r)
        rcp[h, c] = r
        r_buf[h % NS, rs, :] = jnp.broadcast_to(r, (_RC, Dh))

    def pv_round(slot, h, c, dst):
        p = _cat((p_buf[h % NS, c * (NK // 2) + i] for i in range(NK // 2)), 1)
        o = _dot(p, v_ref[slot, h % KC, c * HK:(c + 1) * HK, :])
        if c == 0:
            oacc_ref[...] = o
        else:
            o_buf[dst] = ((o + oacc_ref[...]) * r_buf[h % NS]).astype(o_buf.dtype)

    def kv_start(c):
        k_copy(c).start()
        v_copy(c).start()

    def kv_wait(c):
        k_copy(c).wait()
        v_copy(c).wait()

    def xo_sync(g, n):
        b = g // NG

        @pl.when((g % NG < n) & (b + 1 < B))
        def _():
            x_copy(b + 1).start()

        @pl.when((g % NG >= NG // 2) & (g % NG < NG // 2 + n))
        def _():
            @pl.when(b + 1 < B)
            def _():
                x_copy(b + 1).wait()

            @pl.when(b > 0)
            def _():
                out_copy(b - 1).start()

    def body(G, g0, sync):
        rounds, after = _plan(G, Sq // _RC, ND)
        o_slot = lambda j: LAST if j in (-1, G // 4 - 1) else j
        for d in (mpart, lsum, rcp):
            d.clear()
        for i, ((kind, a, b), chunks) in enumerate(zip(rounds, after)):
            sync(i, kind, a, b)
            if kind == "qk":
                qk_round((g0 + a // KC) % NB, a, b)
            elif kind == "pv":
                pv_round((g0 + a // KC) % NB, a, b, 4 * o_slot(a // 4) + a % 4)
            elif kind == "o":
                o_round(jnp.maximum(g0 + a - 1, 0), o_slot(a - 1), b, True if G % 8 else a == 1, True if G % 8 else a == 0)
            else:
                q_round(jnp.minimum(g0 + a + 1, B * NG - 1), (a + 1) % (G // 4), b)
            for h, c in chunks:
                softmax(g0 < 0, h, c)

    LAST = G // 4 - 1
    CH = G // KC
    RAMP = _RB

    def issued(c):
        return jnp.minimum(c + 2 + jnp.maximum(c - _R0, 0) // 2, RAMP + CH - 1)

    assert (B * NCH - RAMP) % CH == 0 and RAMP % 2 == 0 and CH <= NG // 2
    assert RAMP + 1 + (RAMP - 1 - _R0) // 2 >= RAMP + CH - 1

    def ramp_step(t, _):
        def sync(i, kind, a, b):
            if kind != "qk" or b or a % KC:
                return
            g = 2 * t + a // KC
            kv_wait(g)

            @pl.when(g < NG)
            def _():
                wo_copy(g).wait()

                @pl.when(g + 1 < NG)
                def _():
                    wq_copy(g + 1).wait()

                @pl.when(g + 2 < NG)
                def _():
                    wo_copy(g + 2).start()

                @pl.when(g + 3 < NG)
                def _():
                    wq_copy(g + 3).start()

            for n in (1, 2):
                @pl.when(issued(g - 1) + n <= issued(g))
                def _():
                    kv_start(issued(g - 1) + n)

            if a == 0:
                xo_sync(g + 1, 2)

        body(8, 2 * t, sync)

    def main_step(t, _):
        g0 = RAMP + t * CH

        def sync(i, kind, a, b):
            if i == 0:
                xo_sync(g0 + CH - 1, CH)
                for c in range(CH):
                    kv_wait(g0 + c)
            if kind == "qk" and b == 1 and a % KC == 0:
                c = g0 + CH + a // KC

                @pl.when(c < B * NCH)
                def _():
                    kv_start(c)

        body(G, g0, sync)

    x_copy(0).start()
    wq_copy(0).start()
    kv_start(0)
    wq_copy(1).start()
    wo_copy(0).start()
    o_buf[...] = jnp.zeros_like(o_buf)
    acc_ref[...] = jnp.zeros_like(acc_ref)
    x_copy(0).wait()
    wq_copy(0).wait()
    kv_start(1)
    wq_copy(2).start()
    wo_copy(1).start()
    for n in range(ND):
        q_round(0, 0, n)
    jax.lax.fori_loop(0, RAMP // 2, ramp_step, None)
    jax.lax.fori_loop(0, (B * NCH - RAMP) // CH, main_step, None)
    for n in range(ND):
        o_round(B * NG - 1, LAST, n, False, True)
    out_copy(B - 1).start()
    for b in range(B):
        out_copy(b).wait()


@jax.jit
def pallas_standalone__gqa_block_cached__near_ridge_kernel(x, k_cache, v_cache, wq, wo):
    B, Sq, D = x.shape
    _, Hkv, Sk, Dh = k_cache.shape
    G, NS, NB, KC = _G, _NS, _NB, _KC
    NG, ND, NK = Hkv // 4, D // _L, Sk // _L
    bf16, f32 = jnp.bfloat16, jnp.float32
    DMA = pltpu.SemaphoreType.DMA
    return pl.pallas_call(
        functools.partial(_kernel, G=G),
        in_specs=[pl.BlockSpec(memory_space=pl.ANY)] * 5,
        out_specs=pl.BlockSpec(memory_space=pl.ANY),
        out_shape=jax.ShapeDtypeStruct((B, Sq, D), x.dtype),
        scratch_shapes=[
            pltpu.VMEM(x.shape, x.dtype),
            pltpu.VMEM((NB, KC, Sk, Dh), k_cache.dtype),
            pltpu.VMEM((NB, KC, Sk, Dh), v_cache.dtype),
            pltpu.VMEM(wq.shape, wq.dtype),
            pltpu.VMEM(wo.shape, wo.dtype),
            pltpu.VMEM((B, Sq, D), x.dtype),
            pltpu.VMEM((G, Sq, Dh), bf16),
            pltpu.VMEM((G, Sq, Dh), bf16),
            pltpu.VMEM((ND, Sq, _L), f32),
            pltpu.VMEM((4, Sq, Dh), f32),
            pltpu.VMEM((Sq, Dh), f32),
            pltpu.VMEM((NS, NK, Sq, _L), f32),
            pltpu.VMEM((NS, NK, Sq, _L), bf16),
            pltpu.VMEM((NS, Sq, Dh), f32),
            DMA((B,)), DMA((NB,)), DMA((NB,)), DMA((NG,)), DMA((NG,)), DMA((B,)),
        ],
        compiler_params=pltpu.CompilerParams(
            vmem_limit_bytes=100 * 1024 * 1024,
            disable_bounds_checks=True,
        ),
    )(x, k_cache, v_cache, wq, wo)
```
